```python
import os as _os
_os.environ.setdefault("JAX_PLATFORMS", "cpu")
import jax
import jax.numpy as jnp

def _softmax(x, axis=-1):
    return jax.nn.softmax(x, axis=axis)
def _gelu(x):
    return jax.nn.gelu(x, approximate=True)
def _silu(x):
    return jax.nn.silu(x)
def _sigmoid(x):
    return jax.nn.sigmoid(x)
def _layernorm(x, axis=-1, eps=1e-5):
    m = jnp.mean(x, axis=axis, keepdims=True)
    v = jnp.var(x, axis=axis, keepdims=True)
    return (x - m) / jnp.sqrt(v + eps)
def _scatter_add(tgt, idx, src, axis=0):
    return tgt.at[idx].add(src)
def _segment_sum(src, seg, n):
    return jax.ops.segment_sum(src, seg, n)
class _Rng:
    def __init__(self, key):
        self._k = key
    def _next(self):
        self._k, sub = jax.random.split(self._k)
        return sub
    def normal(self, shape):
        return jax.random.normal(self._next(), shape, dtype=jnp.bfloat16)
    def randint(self, lo, hi, shape):
        return jax.random.randint(self._next(), shape, lo, hi, dtype=jnp.int32)
    def uniform(self, shape, lo=0.0, hi=1.0):
        return jax.random.uniform(self._next(), shape, jnp.bfloat16, lo, hi)
    def permutation(self, n):
        return jax.random.permutation(self._next(), n)


kernel_name = 'gated_mix__linear_attn_block__glu_gated_swiglu__prompt'

def setup_inputs():
    _rng = _Rng(jax.random.key(int.from_bytes(__import__("os").urandom(4), "little")))
    _w = (lambda a: (lambda t: t.astype(jnp.bfloat16) if jnp.issubdtype(t.dtype, jnp.floating) else t)(jnp.asarray(a)))
    def _A_setup():
        B, S, D = 1, 2048, 1024
        return {
            "x": _w((lambda *s: _rng.normal(s) * 0.05)(B, S, D)),
            "wqkv": _w((lambda *s: _rng.normal(s) * 0.8)(D, 3 * D)),
            "wo": _w((lambda *s: _rng.normal(s) * 0.05)(D, D)),
        }
    _A_in = _A_setup()

    def _B_setup():
        B, S, D, F = 1, 2048, 1024, 3584
        return {
            "x": _w((lambda *s: _rng.normal(s) * 0.05)(B, S, D)),
            "w1": _w((lambda *s: _rng.normal(s) * 1.6)(D, F) * (2.0 / D) ** 0.5),
            "w3": _w((lambda *s: _rng.normal(s) * 1.6)(D, F) * (2.0 / D) ** 0.5),
            "w2": _w((lambda *s: _rng.normal(s) * 1.6)(F, D) * (2.0 / F) ** 0.5),
        }
    _B_in = _B_setup()

    return {
        "A_x": _A_in["x"],
        "A_wqkv": _A_in["wqkv"],
        "A_wo": _A_in["wo"],
        "B_x": _B_in["x"],
        "B_w1": _B_in["w1"],
        "B_w3": _B_in["w3"],
        "B_w2": _B_in["w2"],
        "gate_w": _w((lambda *s: _rng.normal(s) * 0.05)(1024) * 16.0),
    }

def reference(A_x, A_wqkv, A_wo, B_x, B_w1, B_w3, B_w2, gate_w):
    def _A_ref(x, wqkv, wo):
        B, S, D = x.shape
        H = 32; Dh = D // H
        qkv = (lambda x, *d: x.transpose(*d))((x @ wqkv).reshape(B, S, 3, H, Dh), 2, 0, 3, 1, 4)
        q, k, v = qkv[0], qkv[1], qkv[2]
        phi = lambda t: jnp.where(t > 0, t + 1, jnp.exp(t)) + 1e-6
        pq, pk = phi(q), phi(k)
        kv = jnp.einsum("bhsd,bhse->bhde", pk, v)
        z = jnp.einsum("bhsd->bhd", pk)
        num = jnp.einsum("bhqd,bhde->bhqe", pq, kv)
        den = jnp.einsum("bhqd,bhd->bhq", pq, z)[..., None] + 1e-6
        o = num / den
        return (lambda x, *d: x.transpose(*d))(o, 0, 2, 1, 3).reshape(B, S, D) @ wo

    def _B_ref(x, w1, w3, w2):
        gate = jnp.einsum("bsd,df->bsf", x, w1)
        up = jnp.einsum("bsd,df->bsf", x, w3)
        h = _silu(gate) * up
        out = jnp.einsum("bsf,fd->bsd", h, w2)
        return out

    x = A_x
    g = _sigmoid((x * gate_w).sum(-1, keepdims=True))
    a = _A_ref(x, A_wqkv, A_wo)
    b = _B_ref(x, B_w1, B_w3, B_w2)
    return g * a + (1 - g) * b
```

```python
import jax
import jax.numpy as jnp
from jax import lax
import jax.experimental.pallas as pl
import jax.experimental.pallas.tpu as pltpu

_S, _D, _F = 2048, 1024, 3584
_H = 32
_DH = _D // _H
_LB = 128
_NB = _D // _LB

_TM1 = 256
_TM = 256
_TF = 512
_NK = 4
_NS = 2
_EPS = 1e-6

_BF = jnp.bfloat16
_F32 = jnp.float32


def _phi(t):
    return jnp.where(t > 0, t + (1.0 + _EPS), jnp.exp(t) + _EPS)


def _dot(a, b):
    return jnp.dot(a, b, preferred_element_type=_F32)


def _dot_tn(a, b):
    return lax.dot_general(a, b, (((0,), (0,)), ((), ())), preferred_element_type=_F32)


def _bf(a):
    return a.astype(_BF)


def _kernel(x_hbm, wqkv_hbm, wo_hbm, w1_hbm, w3_hbm, w2_hbm, gw_hbm, out_hbm,
            x_v, wq_v, wk_v, wv_v, wo_v, w1_v, w3_v, w2_v, gw_v,
            g_v, m_v, z_v, a_v, acc_v, out_v,
            sem_x, sem_k, sem_w, sem_o):
    n1, n2, nf = _S // _TM1, _S // _TM, _F // _TF
    kc, ns = _D // _NK, _D // _NS

    def x_copy(i):
        rows = pl.ds(i * _TM1, _TM1)
        return pltpu.make_async_copy(x_hbm.at[rows, :], x_v.at[rows, :], sem_x.at[i])

    def k_copy(c):
        return pltpu.make_async_copy(wqkv_hbm.at[:, pl.ds(_D + c * kc, kc)],
                                     wk_v.at[:, pl.ds(c * kc, kc)], sem_k.at[c])

    def o_copy(i, s):
        rows, cols = pl.ds(i * _TM, _TM), pl.ds(s * ns, ns)
        return pltpu.make_async_copy(out_v.at[rows, cols], out_hbm.at[rows, cols],
                                     sem_o.at[i * _NS + s])

    cq = pltpu.make_async_copy(wqkv_hbm.at[:, pl.ds(0, _D)], wq_v, sem_w.at[0])
    cv = pltpu.make_async_copy(wqkv_hbm.at[:, pl.ds(2 * _D, _D)], wv_v, sem_w.at[1])
    co = pltpu.make_async_copy(wo_hbm, wo_v, sem_w.at[2])
    c1 = pltpu.make_async_copy(w1_hbm, w1_v, sem_w.at[3])
    c3 = pltpu.make_async_copy(w3_hbm, w3_v, sem_w.at[4])
    c2 = pltpu.make_async_copy(w2_hbm, w2_v, sem_w.at[5])
    cg = pltpu.make_async_copy(gw_hbm, gw_v, sem_w.at[6])

    x_copy(0).start()
    for c in range(_NK):
        k_copy(c).start()
    for i in range(1, n1):
        x_copy(i).start(priority=1)
    for cp in (cg, cv, co, cq, c1, c3, c2):
        cp.start(priority=1)

    def p1_tail(k, xi, first):
        pk = jnp.where(k > 0, k + 1.0, jnp.exp(k)) + _EPS
        d = _dot_tn(_bf(pk), xi)
        if first:
            g_v[...] = d
        else:
            g_v[...] += d
        return jnp.sum(pk, axis=0, keepdims=True)

    def p1_body(i, z):
        r0 = pl.multiple_of(i * _TM1, _TM1)
        x_copy(i).wait()
        xi = x_v[pl.ds(r0, _TM1), :]
        return z + p1_tail(_dot(xi, wk_v[...]), xi, False)

    x_copy(0).wait()
    x0 = x_v[0:_TM1, :]
    ks = []
    for c in range(_NK):
        k_copy(c).wait()
        ks.append(_dot(x0, wk_v[:, c * kc:(c + 1) * kc]))
    z = p1_tail(jnp.concatenate(ks, axis=1), x0, True)
    z = lax.fori_loop(1, n1, p1_body, z)

    cv.wait()
    co.wait()
    same_head = (lax.broadcasted_iota(jnp.int32, (_LB, _LB), 0) // _DH
                 == lax.broadcasted_iota(jnp.int32, (_LB, _LB), 1) // _DH)
    for j in range(_NB):
        sl = slice(j * _LB, (j + 1) * _LB)
        kv = _dot(_bf(g_v[sl, :]), wv_v[:, sl])
        kv = _bf(jnp.where(same_head, kv, 0.0))
        m_v[sl, :] = _bf(_dot(kv, wo_v[sl, :]))
    z_v[...] = jnp.broadcast_to(z, (8, _D))
    cg.wait()
    cq.wait()
    c1.wait()
    c3.wait()
    c2.wait()

    def p2_body(i, carry):
        r0 = pl.multiple_of(i * _TM, _TM)
        xi = x_v[pl.ds(r0, _TM), :]

        pq = _phi(_dot(xi, wq_v[...]))
        lane_head = lax.broadcasted_iota(jnp.int32, (_TM, _LB), 1) // _DH
        dens = []
        for j in range(_NB):
            sl = slice(j * _LB, (j + 1) * _LB)
            t = pq[:, sl] * z_v[0:1, sl]
            dj = None
            for hh in range(_LB // _DH):
                m = lane_head == hh
                sh = jnp.sum(jnp.where(m, t, 0.0), axis=-1, keepdims=True)
                dj = jnp.broadcast_to(sh, (_TM, _LB)) if dj is None else jnp.where(m, sh, dj)
            dens.append(dj)
        den = jnp.concatenate(dens, axis=1) + _EPS
        pqn = _bf(pq * pl.reciprocal(den, approx=False, full_range=False))
        a_v[...] = _dot(pqn, m_v[...])

        for c in range(nf):
            cs = slice(c * _TF, (c + 1) * _TF)
            gate = _dot(xi, w1_v[:, cs])
            up = _dot(xi, w3_v[:, cs])
            hg = 0.5 * gate
            h = _bf((hg * jnp.tanh(hg) + hg) * up)
            if c == 0:
                acc_v[...] = _dot(h, w2_v[cs, :])
            elif c < nf - 1:
                acc_v[...] += _dot(h, w2_v[cs, :])
            else:
                lg = 0.0
                for j in range(_NB):
                    lg = lg + (xi[:, j * _LB:(j + 1) * _LB].astype(_F32)
                               * gw_v[j:j + 1, :].astype(_F32))
                g = jax.nn.sigmoid(jnp.sum(lg, axis=-1, keepdims=True))
                for s in range(_NS):
                    sl = slice(s * ns, (s + 1) * ns)
                    b = acc_v[:, sl] + _dot(h, w2_v[cs, sl])
                    out_v[pl.ds(r0, _TM), sl] = _bf(g * a_v[:, sl] + (1.0 - g) * b)
                    o_copy(i, s).start()
        return carry

    lax.fori_loop(0, n2, p2_body, 0)
    for i in range(n2):
        for s in range(_NS):
            o_copy(i, s).wait()


@jax.jit
def pallas_gated_mix__linear_attn_block__glu_gated_swiglu__prompt_kernel(
    A_x: jax.Array,
    A_wqkv: jax.Array,
    A_wo: jax.Array,
    B_x: jax.Array,
    B_w1: jax.Array,
    B_w3: jax.Array,
    B_w2: jax.Array,
    gate_w: jax.Array,
):
    del B_x
    in_hbm = pl.BlockSpec(memory_space=pl.ANY)
    vmem = pltpu.VMEM
    dma = pltpu.SemaphoreType.DMA
    out = pl.pallas_call(
        _kernel,
        out_shape=jax.ShapeDtypeStruct((_S, _D), _BF),
        in_specs=[in_hbm] * 7,
        out_specs=in_hbm,
        scratch_shapes=[
            vmem((_S, _D), _BF),
            vmem((_D, _D), _BF),
            vmem((_D, _D), _BF),
            vmem((_D, _D), _BF),
            vmem((_D, _D), _BF),
            vmem((_D, _F), _BF),
            vmem((_D, _F), _BF),
            vmem((_F, _D), _BF),
            vmem((_NB, _LB), _BF),
            vmem((_D, _D), _F32),
            vmem((_D, _D), _BF),
            vmem((8, _D), _F32),
            vmem((_TM, _D), _F32),
            vmem((_TM, _D), _F32),
            vmem((_S, _D), _BF),
            dma((_S // _TM1,)),
            dma((_NK,)),
            dma((7,)),
            dma((_S // _TM * _NS,)),
        ],
        compiler_params=pltpu.CompilerParams(vmem_limit_bytes=100 * 1024 * 1024),
    )(A_x.reshape(_S, _D), A_wqkv, A_wo, B_w1, B_w3, B_w2, gate_w.reshape(_NB, _LB))
    return out.reshape(A_x.shape)
```

```python
import jax
import jax.numpy as jnp
from jax import lax
import jax.experimental.pallas as pl
import jax.experimental.pallas.tpu as pltpu

_S, _D, _F = 2048, 1024, 3584
_H = 32
_DH = _D // _H
_LB = 128
_NB = _D // _LB

_TM1 = 256
_TM = 256
_TF = 1792
_AK = 4
_NK = 4
_NS = 2
_EPS = 1e-6

_BF = jnp.bfloat16
_F32 = jnp.float32


def _phi(t):
    return jnp.where(t > 0, t + (1.0 + _EPS), jnp.exp(t) + _EPS)


def _dot(a, b):
    return jnp.dot(a, b, preferred_element_type=_F32)


def _dot_tn(a, b):
    return lax.dot_general(a, b, (((0,), (0,)), ((), ())), preferred_element_type=_F32)


def _bf(a):
    return a.astype(_BF)


def _kernel(x_hbm, wqkv_hbm, wo_hbm, w1_hbm, w3_hbm, w2_hbm, gw_hbm, out_hbm,
            x_v, wq_v, wk_v, wv_v, wo_v, w1_v, w3_v, w2_v, gw_v,
            g_v, m_v, z_v, a_v, acc_v, out_v,
            sem_x, sem_k, sem_w, sem_o):
    n1, n2, nf = _S // _TM1, _S // _TM, _F // _TF
    kc, ns = _D // _NK, _D // _NS

    def x_copy(i):
        rows = pl.ds(i * _TM1, _TM1)
        return pltpu.make_async_copy(x_hbm.at[rows, :], x_v.at[rows, :], sem_x.at[i])

    def k_copy(c):
        return pltpu.make_async_copy(wqkv_hbm.at[:, pl.ds(_D + c * kc, kc)],
                                     wk_v.at[:, pl.ds(c * kc, kc)], sem_k.at[c])

    def o_copy(i, s):
        rows, cols = pl.ds(i * _TM, _TM), pl.ds(s * ns, ns)
        return pltpu.make_async_copy(out_v.at[rows, cols], out_hbm.at[rows, cols],
                                     sem_o.at[i * _NS + s])

    cq = pltpu.make_async_copy(wqkv_hbm.at[:, pl.ds(0, _D)], wq_v, sem_w.at[0])
    cv = pltpu.make_async_copy(wqkv_hbm.at[:, pl.ds(2 * _D, _D)], wv_v, sem_w.at[1])
    co = pltpu.make_async_copy(wo_hbm, wo_v, sem_w.at[2])
    c1 = pltpu.make_async_copy(w1_hbm, w1_v, sem_w.at[3])
    c3 = pltpu.make_async_copy(w3_hbm, w3_v, sem_w.at[4])
    c2 = pltpu.make_async_copy(w2_hbm, w2_v, sem_w.at[5])
    cg = pltpu.make_async_copy(gw_hbm, gw_v, sem_w.at[6])

    x_copy(0).start()
    for c in range(_NK):
        k_copy(c).start()
    for i in range(1, n1):
        x_copy(i).start(priority=1)
    for cp in (cg, cv, co, cq, c1, c3, c2):
        cp.start(priority=1)

    def p1_tail(k, xi, first):
        pk = jnp.where(k > 0, k + 1.0, jnp.exp(k)) + _EPS
        d = _dot_tn(_bf(pk), xi)
        if first:
            g_v[...] = d
        else:
            g_v[...] += d
        return jnp.sum(pk, axis=0, keepdims=True)

    def p1_body(i, z):
        r0 = pl.multiple_of(i * _TM1, _TM1)
        x_copy(i).wait()
        xi = x_v[pl.ds(r0, _TM1), :]
        return z + p1_tail(_dot(xi, wk_v[...]), xi, False)

    x_copy(0).wait()
    x0 = x_v[0:_TM1, :]
    ks = []
    for c in range(_NK):
        k_copy(c).wait()
        ks.append(_dot(x0, wk_v[:, c * kc:(c + 1) * kc]))
    z = p1_tail(jnp.concatenate(ks, axis=1), x0, True)
    z = lax.fori_loop(1, n1, p1_body, z)

    cv.wait()
    co.wait()
    same_head = (lax.broadcasted_iota(jnp.int32, (_LB, _LB), 0) // _DH
                 == lax.broadcasted_iota(jnp.int32, (_LB, _LB), 1) // _DH)
    for j in range(_NB):
        sl = slice(j * _LB, (j + 1) * _LB)
        kv = _dot(_bf(g_v[sl, :]), wv_v[:, sl])
        kv = _bf(jnp.where(same_head, kv, 0.0))
        m_v[sl, :] = _bf(_dot(kv, wo_v[sl, :]))
    z_v[...] = jnp.broadcast_to(z, (8, _D))
    cg.wait()
    cq.wait()
    c1.wait()
    c3.wait()
    c2.wait()

    def p2_body(i, carry):
        r0 = pl.multiple_of(i * _TM, _TM)
        xi = x_v[pl.ds(r0, _TM), :]

        pq = _phi(_dot(xi, wq_v[...]))
        lane_head = lax.broadcasted_iota(jnp.int32, (_TM, _LB), 1) // _DH
        dens = []
        for j in range(_NB):
            sl = slice(j * _LB, (j + 1) * _LB)
            t = pq[:, sl] * z_v[0:1, sl]
            dj = None
            for hh in range(_LB // _DH):
                m = lane_head == hh
                sh = jnp.sum(jnp.where(m, t, 0.0), axis=-1, keepdims=True)
                dj = jnp.broadcast_to(sh, (_TM, _LB)) if dj is None else jnp.where(m, sh, dj)
            dens.append(dj)
        den = jnp.concatenate(dens, axis=1) + _EPS
        pqn = _bf(pq * pl.reciprocal(den, approx=False, full_range=False))

        for c in range(nf):
            cs = slice(c * _TF, (c + 1) * _TF)
            gate = _dot(xi, w1_v[:, cs])
            up = _dot(xi, w3_v[:, cs])
            hg = 0.5 * gate
            h = _bf((hg * jnp.tanh(hg) + hg) * up)
            if c == 0:
                acc_v[...] = _dot(h, w2_v[cs, :])
                ak = _D // _AK
                a_v[...] = sum(_dot(pqn[:, t * ak:(t + 1) * ak], m_v[t * ak:(t + 1) * ak, :])
                               for t in range(_AK))
            elif c < nf - 1:
                acc_v[...] += _dot(h, w2_v[cs, :])
            else:
                lg = 0.0
                for j in range(_NB):
                    lg = lg + (xi[:, j * _LB:(j + 1) * _LB].astype(_F32)
                               * gw_v[j:j + 1, :].astype(_F32))
                g = jax.nn.sigmoid(jnp.sum(lg, axis=-1, keepdims=True))
                for s in range(_NS):
                    sl = slice(s * ns, (s + 1) * ns)
                    b = acc_v[:, sl] + _dot(h, w2_v[cs, sl])
                    out_v[pl.ds(r0, _TM), sl] = _bf(g * a_v[:, sl] + (1.0 - g) * b)
                    o_copy(i, s).start()
        return carry

    lax.fori_loop(0, n2, p2_body, 0)
    for i in range(n2):
        for s in range(_NS):
            o_copy(i, s).wait()


@jax.jit
def pallas_gated_mix__linear_attn_block__glu_gated_swiglu__prompt_kernel(
    A_x: jax.Array,
    A_wqkv: jax.Array,
    A_wo: jax.Array,
    B_x: jax.Array,
    B_w1: jax.Array,
    B_w3: jax.Array,
    B_w2: jax.Array,
    gate_w: jax.Array,
):
    del B_x
    in_hbm = pl.BlockSpec(memory_space=pl.ANY)
    vmem = pltpu.VMEM
    dma = pltpu.SemaphoreType.DMA
    out = pl.pallas_call(
        _kernel,
        out_shape=jax.ShapeDtypeStruct((_S, _D), _BF),
        in_specs=[in_hbm] * 7,
        out_specs=in_hbm,
        scratch_shapes=[
            vmem((_S, _D), _BF),
            vmem((_D, _D), _BF),
            vmem((_D, _D), _BF),
            vmem((_D, _D), _BF),
            vmem((_D, _D), _BF),
            vmem((_D, _F), _BF),
            vmem((_D, _F), _BF),
            vmem((_F, _D), _BF),
            vmem((_NB, _LB), _BF),
            vmem((_D, _D), _F32),
            vmem((_D, _D), _BF),
            vmem((8, _D), _F32),
            vmem((_TM, _D), _F32),
            vmem((_TM, _D), _F32),
            vmem((_S, _D), _BF),
            dma((_S // _TM1,)),
            dma((_NK,)),
            dma((7,)),
            dma((_S // _TM * _NS,)),
        ],
        compiler_params=pltpu.CompilerParams(vmem_limit_bytes=100 * 1024 * 1024),
    )(A_x.reshape(_S, _D), A_wqkv, A_wo, B_w1, B_w3, B_w2, gate_w.reshape(_NB, _LB))
    return out.reshape(A_x.shape)
```

```python
import jax
import jax.numpy as jnp
from jax import lax
import jax.experimental.pallas as pl
import jax.experimental.pallas.tpu as pltpu

_S, _D, _F = 2048, 1024, 3584
_H = 32
_DH = _D // _H
_LB = 128
_NB = _D // _LB

_TM1 = 256
_TM = 256
_TF = 1792
_AK = 4
_NK = 4
_NS = 2
_EPS = 1e-6

_BF = jnp.bfloat16
_F32 = jnp.float32


def _phi(t):
    return jnp.where(t > 0, t + (1.0 + _EPS), jnp.exp(t) + _EPS)


def _dot(a, b):
    return jnp.dot(a, b, preferred_element_type=_F32)


def _dot_tn(a, b):
    return lax.dot_general(a, b, (((0,), (0,)), ((), ())), preferred_element_type=_F32)


def _bf(a):
    return a.astype(_BF)


def _kernel(x_hbm, wqkv_hbm, wo_hbm, w1_hbm, w3_hbm, w2_hbm, gw_hbm, out_hbm,
            x_v, wq_v, wk_v, wv_v, wo_v, w1_v, w3_v, w2_v, gw_v,
            g_v, m_v, z_v, a_v, acc_v, out_v,
            sem_x, sem_k, sem_w, sem_o):
    n1, n2, nf = _S // _TM1, _S // _TM, _F // _TF
    kc, ns = _D // _NK, _D // _NS

    def x_copy(i):
        rows = pl.ds(i * _TM1, _TM1)
        return pltpu.make_async_copy(x_hbm.at[rows, :], x_v.at[rows, :], sem_x.at[i])

    def k_copy(c):
        return pltpu.make_async_copy(wqkv_hbm.at[:, pl.ds(_D + c * kc, kc)],
                                     wk_v.at[:, pl.ds(c * kc, kc)], sem_k.at[c])

    def o_copy(i, s):
        rows, cols = pl.ds(i * _TM, _TM), pl.ds(s * ns, ns)
        return pltpu.make_async_copy(out_v.at[rows, cols], out_hbm.at[rows, cols],
                                     sem_o.at[i * _NS + s])

    cq = pltpu.make_async_copy(wqkv_hbm.at[:, pl.ds(0, _D)], wq_v, sem_w.at[0])
    cv = pltpu.make_async_copy(wqkv_hbm.at[:, pl.ds(2 * _D, _D)], wv_v, sem_w.at[1])
    co = pltpu.make_async_copy(wo_hbm, wo_v, sem_w.at[2])
    c1 = pltpu.make_async_copy(w1_hbm, w1_v, sem_w.at[3])
    c3 = pltpu.make_async_copy(w3_hbm, w3_v, sem_w.at[4])
    c2 = pltpu.make_async_copy(w2_hbm, w2_v, sem_w.at[5])
    cg = pltpu.make_async_copy(gw_hbm, gw_v, sem_w.at[6])

    x_copy(0).start()
    for c in range(_NK):
        k_copy(c).start()
    for i in range(1, n1):
        x_copy(i).start(priority=1)
    for cp in (cg, cv, co, cq, c1, c3, c2):
        cp.start(priority=1)

    def p1_tail(k, xi, first):
        pk = jnp.where(k > 0, k + 1.0, jnp.exp(k)) + _EPS
        d = _dot_tn(_bf(pk), xi)
        if first:
            g_v[...] = d
        else:
            g_v[...] += d
        return jnp.sum(pk, axis=0, keepdims=True)

    def p1_body(i, z):
        r0 = pl.multiple_of(i * _TM1, _TM1)
        x_copy(i).wait()
        xi = x_v[pl.ds(r0, _TM1), :]
        return z + p1_tail(_dot(xi, wk_v[...]), xi, False)

    x_copy(0).wait()
    x0 = x_v[0:_TM1, :]
    ks = []
    for c in range(_NK):
        k_copy(c).wait()
        ks.append(_dot(x0, wk_v[:, c * kc:(c + 1) * kc]))
    z = p1_tail(jnp.concatenate(ks, axis=1), x0, True)
    z = lax.fori_loop(1, n1, p1_body, z)

    cv.wait()
    co.wait()
    same_head = (lax.broadcasted_iota(jnp.int32, (_LB, _LB), 0) // _DH
                 == lax.broadcasted_iota(jnp.int32, (_LB, _LB), 1) // _DH)
    blocks = [slice(j * _LB, (j + 1) * _LB) for j in range(_NB)]
    kvs = [_bf(jnp.where(same_head, _dot(_bf(g_v[sl, :]), wv_v[:, sl]), 0.0)) for sl in blocks]
    for sl, kv in zip(blocks, kvs):
        m_v[sl, :] = _bf(_dot(kv, wo_v[sl, :]))
    z_v[...] = jnp.broadcast_to(z, (8, _D))
    cg.wait()
    cq.wait()
    c1.wait()
    c3.wait()
    c2.wait()

    def p2_body(i, carry):
        r0 = pl.multiple_of(i * _TM, _TM)
        xi = x_v[pl.ds(r0, _TM), :]

        pq = _phi(_dot(xi, wq_v[...]))
        lane_head = lax.broadcasted_iota(jnp.int32, (_TM, _LB), 1) // _DH
        dens = []
        for j in range(_NB):
            sl = slice(j * _LB, (j + 1) * _LB)
            t = pq[:, sl] * z_v[0:1, sl]
            dj = None
            for hh in range(_LB // _DH):
                m = lane_head == hh
                sh = jnp.sum(jnp.where(m, t, 0.0), axis=-1, keepdims=True)
                dj = jnp.broadcast_to(sh, (_TM, _LB)) if dj is None else jnp.where(m, sh, dj)
            dens.append(dj)
        den = jnp.concatenate(dens, axis=1) + _EPS
        pqn = _bf(pq * pl.reciprocal(den, approx=False, full_range=False))

        for c in range(nf):
            cs = slice(c * _TF, (c + 1) * _TF)
            gate = _dot(xi, w1_v[:, cs])
            up = _dot(xi, w3_v[:, cs])
            hg = 0.5 * gate
            h = _bf((hg * jnp.tanh(hg) + hg) * up)
            if c == 0:
                acc_v[...] = _dot(h, w2_v[cs, :])
                ak = _D // _AK
                a_v[...] = sum(_dot(pqn[:, t * ak:(t + 1) * ak], m_v[t * ak:(t + 1) * ak, :])
                               for t in range(_AK))
            elif c < nf - 1:
                acc_v[...] += _dot(h, w2_v[cs, :])
            else:
                lg = 0.0
                for j in range(_NB):
                    lg = lg + (xi[:, j * _LB:(j + 1) * _LB].astype(_F32)
                               * gw_v[j:j + 1, :].astype(_F32))
                g = jax.nn.sigmoid(jnp.sum(lg, axis=-1, keepdims=True))
                for s in range(_NS):
                    sl = slice(s * ns, (s + 1) * ns)
                    b = acc_v[:, sl] + _dot(h, w2_v[cs, sl])
                    out_v[pl.ds(r0, _TM), sl] = _bf(g * a_v[:, sl] + (1.0 - g) * b)
                    o_copy(i, s).start()
        return carry

    lax.fori_loop(0, n2, p2_body, 0)
    for i in range(n2):
        for s in range(_NS):
            o_copy(i, s).wait()


@jax.jit
def pallas_gated_mix__linear_attn_block__glu_gated_swiglu__prompt_kernel(
    A_x: jax.Array,
    A_wqkv: jax.Array,
    A_wo: jax.Array,
    B_x: jax.Array,
    B_w1: jax.Array,
    B_w3: jax.Array,
    B_w2: jax.Array,
    gate_w: jax.Array,
):
    del B_x
    in_hbm = pl.BlockSpec(memory_space=pl.ANY)
    vmem = pltpu.VMEM
    dma = pltpu.SemaphoreType.DMA
    out = pl.pallas_call(
        _kernel,
        out_shape=jax.ShapeDtypeStruct((_S, _D), _BF),
        in_specs=[in_hbm] * 7,
        out_specs=in_hbm,
        scratch_shapes=[
            vmem((_S, _D), _BF),
            vmem((_D, _D), _BF),
            vmem((_D, _D), _BF),
            vmem((_D, _D), _BF),
            vmem((_D, _D), _BF),
            vmem((_D, _F), _BF),
            vmem((_D, _F), _BF),
            vmem((_F, _D), _BF),
            vmem((_NB, _LB), _BF),
            vmem((_D, _D), _F32),
            vmem((_D, _D), _BF),
            vmem((8, _D), _F32),
            vmem((_TM, _D), _F32),
            vmem((_TM, _D), _F32),
            vmem((_S, _D), _BF),
            dma((_S // _TM1,)),
            dma((_NK,)),
            dma((7,)),
            dma((_S // _TM * _NS,)),
        ],
        compiler_params=pltpu.CompilerParams(vmem_limit_bytes=100 * 1024 * 1024),
    )(A_x.reshape(_S, _D), A_wqkv, A_wo, B_w1, B_w3, B_w2, gate_w.reshape(_NB, _LB))
    return out.reshape(A_x.shape)
```

```python
import jax
import jax.numpy as jnp
from jax import lax
import jax.experimental.pallas as pl
import jax.experimental.pallas.tpu as pltpu

_S, _D, _F = 2048, 1024, 3584
_H = 32
_DH = _D // _H
_LB = 128
_NB = _D // _LB

_T0 = 128
_T1 = 384
_TM = 256
_TF = 512
_AK = 4
_NK = 4
_NS = 2
_EPS = 1e-6

_BF = jnp.bfloat16
_F32 = jnp.float32


def _phi(t):
    return jnp.where(t > 0, t + (1.0 + _EPS), jnp.exp(t) + _EPS)


def _dot(a, b):
    return jnp.dot(a, b, preferred_element_type=_F32)


def _dot_tn(a, b):
    return lax.dot_general(a, b, (((0,), (0,)), ((), ())), preferred_element_type=_F32)


def _bf(a):
    return a.astype(_BF)


def _kernel(x_hbm, wqkv_hbm, wo_hbm, w1_hbm, w3_hbm, w2_hbm, gw_hbm, out_hbm,
            x_v, wq_v, wk_v, wv_v, wo_v, w1_v, w3_v, w2_v, gw_v,
            g_v, m_v, z_v, a_v, acc_v, out_v,
            sem_x, sem_k, sem_w, sem_o):
    n1, n2, nf = (_S - _T0) // _T1, _S // _TM, _F // _TF
    kc, ns = _D // _NK, _D // _NS

    def x_copy(i):
        rows = pl.ds(_T0 + i * _T1, _T1)
        return pltpu.make_async_copy(x_hbm.at[rows, :], x_v.at[rows, :], sem_x.at[i])

    def k_copy(c):
        return pltpu.make_async_copy(wqkv_hbm.at[:, pl.ds(_D + c * kc, kc)],
                                     wk_v.at[:, pl.ds(c * kc, kc)], sem_k.at[c])

    def o_copy(i, s):
        rows, cols = pl.ds(i * _TM, _TM), pl.ds(s * ns, ns)
        return pltpu.make_async_copy(out_v.at[rows, cols], out_hbm.at[rows, cols],
                                     sem_o.at[i * _NS + s])

    cq = pltpu.make_async_copy(wqkv_hbm.at[:, pl.ds(0, _D)], wq_v, sem_w.at[0])
    cv = pltpu.make_async_copy(wqkv_hbm.at[:, pl.ds(2 * _D, _D)], wv_v, sem_w.at[1])
    co = pltpu.make_async_copy(wo_hbm, wo_v, sem_w.at[2])
    c1 = pltpu.make_async_copy(w1_hbm, w1_v, sem_w.at[3])
    c3 = pltpu.make_async_copy(w3_hbm, w3_v, sem_w.at[4])
    c2 = pltpu.make_async_copy(w2_hbm, w2_v, sem_w.at[5])
    cg = pltpu.make_async_copy(gw_hbm, gw_v, sem_w.at[6])
    cx = pltpu.make_async_copy(x_hbm.at[0:_T0, :], x_v.at[0:_T0, :], sem_w.at[7])

    cx.start()
    for c in range(_NK):
        k_copy(c).start()
    for i in range(1, n1):
        x_copy(i).start(priority=1)
    for cp in (cg, cv, co, cq, c1, c3, c2):
        cp.start(priority=1)

    def phi_k(k):
        return jnp.where(k > 0, k + 1.0, jnp.exp(k)) + _EPS

    def p1_body(i, z):
        r0 = pl.multiple_of(_T0 + i * _T1, 128)
        x_copy(i).wait()
        xi = x_v[pl.ds(r0, _T1), :]
        pk = phi_k(_dot(xi, wk_v[...]))
        g_v[...] += _dot_tn(_bf(pk), xi)
        return z + jnp.sum(pk, axis=0, keepdims=True)

    cx.wait()
    x0 = x_v[0:_T0, :]
    pks = []
    for c in range(_NK):
        k_copy(c).wait()
        if c == 1:
            x_copy(0).start()
        pks.append(phi_k(_dot(x0, wk_v[:, c * kc:(c + 1) * kc])))
        if c > 0:
            g_v[(c - 1) * kc:c * kc, :] = _dot_tn(_bf(pks[c - 1]), x0)
    g_v[(_NK - 1) * kc:_NK * kc, :] = _dot_tn(_bf(pks[_NK - 1]), x0)
    z = jnp.sum(jnp.concatenate(pks, axis=1), axis=0, keepdims=True)
    z = lax.fori_loop(0, n1, p1_body, z)

    cv.wait()
    co.wait()
    same_head = (lax.broadcasted_iota(jnp.int32, (_LB, _LB), 0) // _DH
                 == lax.broadcasted_iota(jnp.int32, (_LB, _LB), 1) // _DH)
    blocks = [slice(j * _LB, (j + 1) * _LB) for j in range(_NB)]
    kvs = []
    for j, sl in enumerate(blocks):
        kvs.append(_bf(jnp.where(same_head, _dot(_bf(g_v[sl, :]), wv_v[:, sl]), 0.0)))
        if j > 0:
            m_v[blocks[j - 1], :] = _bf(_dot(kvs[j - 1], wo_v[blocks[j - 1], :]))
    m_v[blocks[-1], :] = _bf(_dot(kvs[-1], wo_v[blocks[-1], :]))
    z_v[...] = jnp.broadcast_to(z, (8, _D))
    cg.wait()
    cq.wait()
    c1.wait()
    c3.wait()
    c2.wait()

    def p2_body(i, carry):
        r0 = pl.multiple_of(i * _TM, _TM)
        xi = x_v[pl.ds(r0, _TM), :]

        pq = _phi(_dot(xi, wq_v[...]))
        lane_head = lax.broadcasted_iota(jnp.int32, (_TM, _LB), 1) // _DH
        dens = []
        for j in range(_NB):
            sl = slice(j * _LB, (j + 1) * _LB)
            t = pq[:, sl] * z_v[0:1, sl]
            dj = None
            for hh in range(_LB // _DH):
                m = lane_head == hh
                sh = jnp.sum(jnp.where(m, t, 0.0), axis=-1, keepdims=True)
                dj = jnp.broadcast_to(sh, (_TM, _LB)) if dj is None else jnp.where(m, sh, dj)
            dens.append(dj)
        den = jnp.concatenate(dens, axis=1) + _EPS
        pqn = _bf(pq * pl.reciprocal(den, approx=False, full_range=False))

        for c in range(nf):
            cs = slice(c * _TF, (c + 1) * _TF)
            gate = _dot(xi, w1_v[:, cs])
            up = _dot(xi, w3_v[:, cs])
            hg = 0.5 * gate
            h = _bf((hg * jnp.tanh(hg) + hg) * up)
            if c == 0:
                acc_v[...] = _dot(h, w2_v[cs, :])
                ak = _D // _AK
                a_v[...] = sum(_dot(pqn[:, t * ak:(t + 1) * ak], m_v[t * ak:(t + 1) * ak, :])
                               for t in range(_AK))
            elif c < nf - 1:
                acc_v[...] += _dot(h, w2_v[cs, :])
            else:
                lg = 0.0
                for j in range(_NB):
                    lg = lg + (xi[:, j * _LB:(j + 1) * _LB].astype(_F32)
                               * gw_v[j:j + 1, :].astype(_F32))
                g = jax.nn.sigmoid(jnp.sum(lg, axis=-1, keepdims=True))
                for s in range(_NS):
                    sl = slice(s * ns, (s + 1) * ns)
                    b = acc_v[:, sl] + _dot(h, w2_v[cs, sl])
                    out_v[pl.ds(r0, _TM), sl] = _bf(g * a_v[:, sl] + (1.0 - g) * b)
                    o_copy(i, s).start()
        return carry

    lax.fori_loop(0, n2, p2_body, 0)
    for i in range(n2):
        for s in range(_NS):
            o_copy(i, s).wait()


@jax.jit
def pallas_gated_mix__linear_attn_block__glu_gated_swiglu__prompt_kernel(
    A_x: jax.Array,
    A_wqkv: jax.Array,
    A_wo: jax.Array,
    B_x: jax.Array,
    B_w1: jax.Array,
    B_w3: jax.Array,
    B_w2: jax.Array,
    gate_w: jax.Array,
):
    del B_x
    in_hbm = pl.BlockSpec(memory_space=pl.ANY)
    vmem = pltpu.VMEM
    dma = pltpu.SemaphoreType.DMA
    out = pl.pallas_call(
        _kernel,
        out_shape=jax.ShapeDtypeStruct((_S, _D), _BF),
        in_specs=[in_hbm] * 7,
        out_specs=in_hbm,
        scratch_shapes=[
            vmem((_S, _D), _BF),
            vmem((_D, _D), _BF),
            vmem((_D, _D), _BF),
            vmem((_D, _D), _BF),
            vmem((_D, _D), _BF),
            vmem((_D, _F), _BF),
            vmem((_D, _F), _BF),
            vmem((_F, _D), _BF),
            vmem((_NB, _LB), _BF),
            vmem((_D, _D), _F32),
            vmem((_D, _D), _BF),
            vmem((8, _D), _F32),
            vmem((_TM, _D), _F32),
            vmem((_TM, _D), _F32),
            vmem((_S, _D), _BF),
            dma(((_S - _T0) // _T1,)),
            dma((_NK,)),
            dma((8,)),
            dma((_S // _TM * _NS,)),
        ],
        compiler_params=pltpu.CompilerParams(vmem_limit_bytes=100 * 1024 * 1024),
    )(A_x.reshape(_S, _D), A_wqkv, A_wo, B_w1, B_w3, B_w2, gate_w.reshape(_NB, _LB))
    return out.reshape(A_x.shape)
```

```python
import jax
import jax.numpy as jnp
from jax import lax
import jax.experimental.pallas as pl
import jax.experimental.pallas.tpu as pltpu

_S, _D, _F = 2048, 1024, 3584
_H = 32
_DH = _D // _H
_LB = 128
_NB = _D // _LB

_T0 = 128
_T1 = 384
_TM = 256
_TF = 512
_AK = 4
_NK = 4
_NS = 2
_EPS = 1e-6

_BF = jnp.bfloat16
_F32 = jnp.float32


def _phi(t):
    return jnp.where(t > 0, t + (1.0 + _EPS), jnp.exp(t) + _EPS)


def _dot(a, b):
    return jnp.dot(a, b, preferred_element_type=_F32)


def _dot_tn(a, b):
    return lax.dot_general(a, b, (((0,), (0,)), ((), ())), preferred_element_type=_F32)


def _bf(a):
    return a.astype(_BF)


def _kernel(x_hbm, wqkv_hbm, wo_hbm, w1_hbm, w3_hbm, w2_hbm, gw_hbm, out_hbm,
            x_v, wq_v, wk_v, wv_v, wo_v, w1_v, w3_v, w2_v, gw_v,
            g_v, m_v, z_v, a_v, acc_v, out_v,
            sem_x, sem_k, sem_w, sem_o):
    n1, n2, nf = (_S - _T0) // _T1, _S // _TM, _F // _TF
    kc, ns = _D // _NK, _D // _NS

    def x_copy(i):
        rows = pl.ds(_T0 + i * _T1, _T1)
        return pltpu.make_async_copy(x_hbm.at[rows, :], x_v.at[rows, :], sem_x.at[i])

    def k_copy(c):
        return pltpu.make_async_copy(wqkv_hbm.at[:, pl.ds(_D + c * kc, kc)],
                                     wk_v.at[:, pl.ds(c * kc, kc)], sem_k.at[c])

    def o_copy(i, s):
        rows, cols = pl.ds(i * _TM, _TM), pl.ds(s * ns, ns)
        return pltpu.make_async_copy(out_v.at[rows, cols], out_hbm.at[rows, cols],
                                     sem_o.at[i * _NS + s])

    cq = pltpu.make_async_copy(wqkv_hbm.at[:, pl.ds(0, _D)], wq_v, sem_w.at[0])
    cv = pltpu.make_async_copy(wqkv_hbm.at[:, pl.ds(2 * _D, _D)], wv_v, sem_w.at[1])
    co = pltpu.make_async_copy(wo_hbm, wo_v, sem_w.at[2])
    c1 = pltpu.make_async_copy(w1_hbm, w1_v, sem_w.at[3])
    c3 = pltpu.make_async_copy(w3_hbm, w3_v, sem_w.at[4])
    c2 = pltpu.make_async_copy(w2_hbm, w2_v, sem_w.at[5])
    cg = pltpu.make_async_copy(gw_hbm, gw_v, sem_w.at[6])
    cx = pltpu.make_async_copy(x_hbm.at[0:_T0, :], x_v.at[0:_T0, :], sem_w.at[7])

    cx.start()
    for c in range(_NK):
        k_copy(c).start()
    for i in range(1, n1):
        x_copy(i).start(priority=1)
    for cp in (cg, cv, co, cq, c1, c3, c2):
        cp.start(priority=1)

    def phi_k(k):
        return jnp.where(k > 0, k + 1.0, jnp.exp(k)) + _EPS

    def p1_body(i, z):
        r0 = pl.multiple_of(_T0 + i * _T1, 128)
        x_copy(i).wait()
        xi = x_v[pl.ds(r0, _T1), :]
        pk = phi_k(_dot(xi, wk_v[...]))
        g_v[...] += _dot_tn(_bf(pk), xi)
        return z + jnp.sum(pk, axis=0, keepdims=True)

    cx.wait()
    pks = []
    for c in range(_NK):
        k_copy(c).wait()
        if c == 1:
            x_copy(0).start()
        pks.append(phi_k(_dot(x_v[0:_T0, :], wk_v[:, c * kc:(c + 1) * kc])))
        if c > 0:
            g_v[(c - 1) * kc:c * kc, :] = _dot_tn(_bf(pks[c - 1]), x_v[0:_T0, :])
    g_v[(_NK - 1) * kc:_NK * kc, :] = _dot_tn(_bf(pks[_NK - 1]), x_v[0:_T0, :])
    z = jnp.sum(jnp.concatenate(pks, axis=1), axis=0, keepdims=True)
    z = lax.fori_loop(0, n1, p1_body, z)

    cv.wait()
    co.wait()
    same_head = (lax.broadcasted_iota(jnp.int32, (_LB, _LB), 0) // _DH
                 == lax.broadcasted_iota(jnp.int32, (_LB, _LB), 1) // _DH)
    blocks = [slice(j * _LB, (j + 1) * _LB) for j in range(_NB)]
    kvs = []
    for j, sl in enumerate(blocks):
        kvs.append(_bf(jnp.where(same_head, _dot(_bf(g_v[sl, :]), wv_v[:, sl]), 0.0)))
        if j > 0:
            m_v[blocks[j - 1], :] = _bf(_dot(kvs[j - 1], wo_v[blocks[j - 1], :]))
    m_v[blocks[-1], :] = _bf(_dot(kvs[-1], wo_v[blocks[-1], :]))
    z_v[...] = jnp.broadcast_to(z, (8, _D))
    cg.wait()
    cq.wait()
    c1.wait()
    c3.wait()
    c2.wait()

    def p2_body(i, carry):
        r0 = pl.multiple_of(i * _TM, _TM)
        xi = x_v[pl.ds(r0, _TM), :]

        pq = _phi(_dot(xi, wq_v[...]))
        lane_head = lax.broadcasted_iota(jnp.int32, (_TM, _LB), 1) // _DH
        dens = []
        for j in range(_NB):
            sl = slice(j * _LB, (j + 1) * _LB)
            t = pq[:, sl] * z_v[0:1, sl]
            dj = None
            for hh in range(_LB // _DH):
                m = lane_head == hh
                sh = jnp.sum(jnp.where(m, t, 0.0), axis=-1, keepdims=True)
                dj = jnp.broadcast_to(sh, (_TM, _LB)) if dj is None else jnp.where(m, sh, dj)
            dens.append(dj)
        den = jnp.concatenate(dens, axis=1) + _EPS
        pqn = _bf(pq * pl.reciprocal(den, approx=False, full_range=False))

        for c in range(nf):
            cs = slice(c * _TF, (c + 1) * _TF)
            gate = _dot(xi, w1_v[:, cs])
            up = _dot(xi, w3_v[:, cs])
            hg = 0.5 * gate
            h = _bf((hg * jnp.tanh(hg) + hg) * up)
            if c == 0:
                acc_v[...] = _dot(h, w2_v[cs, :])
                ak = _D // _AK
                a_v[...] = sum(_dot(pqn[:, t * ak:(t + 1) * ak], m_v[t * ak:(t + 1) * ak, :])
                               for t in range(_AK))
            elif c < nf - 1:
                acc_v[...] += _dot(h, w2_v[cs, :])
            else:
                lg = 0.0
                for j in range(_NB):
                    lg = lg + (xi[:, j * _LB:(j + 1) * _LB].astype(_F32)
                               * gw_v[j:j + 1, :].astype(_F32))
                g = jax.nn.sigmoid(jnp.sum(lg, axis=-1, keepdims=True))
                for s in range(_NS):
                    sl = slice(s * ns, (s + 1) * ns)
                    b = acc_v[:, sl] + _dot(h, w2_v[cs, sl])
                    out_v[pl.ds(r0, _TM), sl] = _bf(g * a_v[:, sl] + (1.0 - g) * b)
                    o_copy(i, s).start()
        return carry

    lax.fori_loop(0, n2, p2_body, 0)
    for i in range(n2):
        for s in range(_NS):
            o_copy(i, s).wait()


@jax.jit
def pallas_gated_mix__linear_attn_block__glu_gated_swiglu__prompt_kernel(
    A_x: jax.Array,
    A_wqkv: jax.Array,
    A_wo: jax.Array,
    B_x: jax.Array,
    B_w1: jax.Array,
    B_w3: jax.Array,
    B_w2: jax.Array,
    gate_w: jax.Array,
):
    del B_x
    in_hbm = pl.BlockSpec(memory_space=pl.ANY)
    vmem = pltpu.VMEM
    dma = pltpu.SemaphoreType.DMA
    out = pl.pallas_call(
        _kernel,
        out_shape=jax.ShapeDtypeStruct((_S, _D), _BF),
        in_specs=[in_hbm] * 7,
        out_specs=in_hbm,
        scratch_shapes=[
            vmem((_S, _D), _BF),
            vmem((_D, _D), _BF),
            vmem((_D, _D), _BF),
            vmem((_D, _D), _BF),
            vmem((_D, _D), _BF),
            vmem((_D, _F), _BF),
            vmem((_D, _F), _BF),
            vmem((_F, _D), _BF),
            vmem((_NB, _LB), _BF),
            vmem((_D, _D), _F32),
            vmem((_D, _D), _BF),
            vmem((8, _D), _F32),
            vmem((_TM, _D), _F32),
            vmem((_TM, _D), _F32),
            vmem((_S, _D), _BF),
            dma(((_S - _T0) // _T1,)),
            dma((_NK,)),
            dma((8,)),
            dma((_S // _TM * _NS,)),
        ],
        compiler_params=pltpu.CompilerParams(vmem_limit_bytes=100 * 1024 * 1024),
    )(A_x.reshape(_S, _D), A_wqkv, A_wo, B_w1, B_w3, B_w2, gate_w.reshape(_NB, _LB))
    return out.reshape(A_x.shape)
```
